```python
import os as _os
_os.environ.setdefault("JAX_PLATFORMS", "cpu")
import jax
import jax.numpy as jnp

def _softmax(x, axis=-1):
    return jax.nn.softmax(x, axis=axis)
def _gelu(x):
    return jax.nn.gelu(x, approximate=True)
def _silu(x):
    return jax.nn.silu(x)
def _sigmoid(x):
    return jax.nn.sigmoid(x)
def _layernorm(x, axis=-1, eps=1e-5):
    m = jnp.mean(x, axis=axis, keepdims=True)
    v = jnp.var(x, axis=axis, keepdims=True)
    return (x - m) / jnp.sqrt(v + eps)
def _scatter_add(tgt, idx, src, axis=0):
    return tgt.at[idx].add(src)
def _segment_sum(src, seg, n):
    return jax.ops.segment_sum(src, seg, n)
class _Rng:
    def __init__(self, key):
        self._k = key
    def _next(self):
        self._k, sub = jax.random.split(self._k)
        return sub
    def normal(self, shape):
        return jax.random.normal(self._next(), shape, dtype=jnp.bfloat16)
    def randint(self, lo, hi, shape):
        return jax.random.randint(self._next(), shape, lo, hi, dtype=jnp.int32)
    def uniform(self, shape, lo=0.0, hi=1.0):
        return jax.random.uniform(self._next(), shape, jnp.bfloat16, lo, hi)
    def permutation(self, n):
        return jax.random.permutation(self._next(), n)


kernel_name = 'concat_heads__grouped_kv_mqa__sliding_block__prompt'

def setup_inputs():
    _rng = _Rng(jax.random.key(int.from_bytes(__import__("os").urandom(4), "little")))
    _w = (lambda a: (lambda t: t.astype(jnp.bfloat16) if jnp.issubdtype(t.dtype, jnp.floating) else t)(jnp.asarray(a)))
    def _A_setup():
        B, S, D, H = 1, 2048, 1024, 32
        Dh = D // H
        return {
            "x": _w((lambda *s: _rng.normal(s) * 0.05)(B, S, D)),
            "wq": _w((lambda *s: _rng.normal(s) * 1.6)(D, H * Dh)),
            "wk": _w((lambda *s: _rng.normal(s) * 1.6)(D, Dh)),
            "wv": _w((lambda *s: _rng.normal(s) * 0.1)(D, Dh)),
            "wo": _w((lambda *s: _rng.normal(s) * 0.1)(H * Dh, D)),
        }
    _A_in = _A_setup()

    def _B_setup():
        B, S, D = 1, 2048, 1024
        return {
            "x": _w((lambda *s: _rng.normal(s) * 0.2)(B, S, D)),
            "wqkv": _w((lambda *s: _rng.normal(s) * 0.2)(D, 3 * D)),
            "wo": _w((lambda *s: _rng.normal(s) * 0.05)(D, D)),
        }
    _B_in = _B_setup()

    return {
        "A_x": _A_in["x"],
        "A_wq": _A_in["wq"],
        "A_wk": _A_in["wk"],
        "A_wv": _A_in["wv"],
        "A_wo": _A_in["wo"],
        "B_x": _B_in["x"],
        "B_wqkv": _B_in["wqkv"],
        "B_wo": _B_in["wo"],
    }

def reference(A_x, A_wq, A_wk, A_wv, A_wo, B_x, B_wqkv, B_wo):
    def _A_ref(x, wq, wk, wv, wo):
        B, S, D = x.shape
        H = 32
        Dh = D // H
        q = (lambda x, *d: x.transpose(*d))((x @ wq).reshape(B, S, H, Dh), 0, 2, 1, 3)
        k = x @ wk
        v = x @ wv
        scores = jnp.einsum("bhqd,bkd->bhqk", q, k) * (Dh ** -0.5)
        p = _softmax(scores, axis=-1)
        o = jnp.einsum("bhqk,bkd->bhqd", p, v)
        return (lambda x, *d: x.transpose(*d))(o, 0, 2, 1, 3).reshape(B, S, H * Dh) @ wo

    def _B_ref(x, wqkv, wo):
        B, S, D = x.shape
        H = 32; Dh = D // H; W = 256
        qkv = (lambda x, *d: x.transpose(*d))((x @ wqkv).reshape(B, S, 3, H, Dh), 2, 0, 3, 1, 4)
        q, k, v = qkv[0], qkv[1], qkv[2]
        scores = jnp.einsum("bhqd,bhkd->bhqk", q, k) * (Dh ** -0.5)
        idx = jnp.arange(S)
        mask = (idx[:, None] - idx[None, :] >= 0) & (idx[:, None] - idx[None, :] < W)
        scores = jnp.where(mask[None, None], scores, -1e9)
        p = _softmax(scores, axis=-1)
        o = jnp.einsum("bhqk,bhkd->bhqd", p, v)
        return (lambda x, *d: x.transpose(*d))(o, 0, 2, 1, 3).reshape(B, S, D) @ wo

    a = _A_ref(A_x, A_wq, A_wk, A_wv, A_wo)
    b = _B_ref(B_x, B_wqkv, B_wo)
    return jnp.concatenate([a, b], axis=-1)
```

```python
import math

import jax
import jax.numpy as jnp
from jax import lax
import jax.experimental.pallas as pl
import jax.experimental.pallas.tpu as pltpu

H = 32
WIN = 256
NEG = -1e9
GH = 4
TA = 1024
KC = 128
RP = 256
XC = 512
TB = 512
QB = 128

_NT = (((1,), (1,)), ((), ()))
_TN = (((0,), (0,)), ((), ()))


def _dot(a, b):
    return jnp.dot(a, b, preferred_element_type=jnp.float32)


def _dot_nt(a, b):
    return lax.dot_general(a, b, _NT, preferred_element_type=jnp.float32)


def _dot_tn(a, b):
    return lax.dot_general(a, b, _TN, preferred_element_type=jnp.float32)


def _kernel(xa_hbm, wq_hbm, wkt_hbm, wvt_hbm, woa_hbm, xb_hbm, wqkv_hbm, wob_hbm,
            o_hbm,
            xa_ref, wq_ref, wkt_ref, wvt_ref, woa_ref, xb_ref, wqkv_ref, wob_ref,
            in_sems, out_sems,
            ks_ref, vta_ref, qa_ref, ota_ref, oa_ref,
            sa_ref, cma_ref, sb_ref, cmb_ref, m_ref, l_ref, acc_ref,
            qm_ref, kb_ref, vtb_ref, otb_ref, ob_ref, mask_ref,
            bsa_ref, bma_ref, bsb_ref, bmb_ref,
            *, S, D):
    dh = D // H
    ng = H // GH
    n_chunks = S // KC
    n_xc = S // XC
    qscale = (dh ** -0.5) * math.log2(math.e)
    bf16 = jnp.bfloat16
    lane128 = lax.broadcasted_iota(jnp.int32, (1, GH * dh), 1)

    first = [pltpu.make_async_copy(wkt_hbm, wkt_ref, in_sems.at[0]),
             pltpu.make_async_copy(wvt_hbm, wvt_ref, in_sems.at[1])]
    xcp = [pltpu.make_async_copy(xa_hbm.at[c * XC:(c + 1) * XC],
                                 xa_ref.at[c * XC:(c + 1) * XC],
                                 in_sems.at[2 + c]) for c in range(n_xc)]
    base = 2 + n_xc
    wq_cp = pltpu.make_async_copy(wq_hbm, wq_ref, in_sems.at[base])
    later = [pltpu.make_async_copy(h, v, in_sems.at[base + 1 + i])
             for i, (h, v) in enumerate(((woa_hbm, woa_ref), (xb_hbm, xb_ref),
                                         (wqkv_hbm, wqkv_ref), (wob_hbm, wob_ref)))]
    for cp in first + xcp + [wq_cp]:
        cp.start()

    row = lax.broadcasted_iota(jnp.int32, (dh, GH * dh), 0)
    col = lax.broadcasted_iota(jnp.int32, (dh, GH * dh), 1)
    for cp in first:
        cp.wait()
    for c in range(n_xc):
        xcp[c].wait()
        xc = xa_ref[c * XC:(c + 1) * XC, :]
        k = _dot_nt(xc, wkt_ref[...]).astype(bf16)
        vt = _dot_nt(wvt_ref[...], xc).astype(bf16)
        for j in range(GH):
            ej = jnp.where(col == row + dh * j, 1.0, 0.0).astype(bf16)
            ks_ref[j, c * XC:(c + 1) * XC, :] = _dot(k, ej).astype(bf16)
        for cc in range(XC // KC):
            vta_ref[c * (XC // KC) + cc] = vt[:, cc * KC:(cc + 1) * KC]
    for cp in later:
        cp.start()
    kb_ref[:, 0:WIN, :] = jnp.zeros((ng, WIN, GH * dh), bf16)
    vtb_ref[:, 0:WIN] = jnp.zeros((D, WIN), bf16)
    m_ref[...] = jnp.full(m_ref.shape, -jnp.inf, jnp.float32)
    l_ref[...] = jnp.zeros(l_ref.shape, jnp.float32)
    acc_ref[...] = jnp.zeros(acc_ref.shape, jnp.float32)
    wq_cp.wait()

    n_it = ng * n_chunks
    bufs = ((sa_ref, cma_ref), (sb_ref, cmb_ref))

    def qk(it, slot, j):
        s_r, cm_r = bufs[slot]
        g = it // n_chunks
        c = it % n_chunks
        kj = ks_ref[j, pl.ds(pl.multiple_of(c * KC, KC), KC), :]
        s = _dot_nt(kj, qa_ref[g])
        s_r[j] = s
        cm_r[j] = jnp.max(s, axis=0, keepdims=True)

    def sm(it, slot, j):
        s_r, cm_r = bufs[slot]
        c = it % n_chunks
        m = m_ref[j]
        m_new = jnp.maximum(m, cm_r[j])
        p = jnp.exp2(s_r[j] - m_new)
        alpha = jnp.exp2(m - m_new)
        l_ref[j] = l_ref[j] * alpha + jnp.sum(p, axis=0, keepdims=True)
        acc_ref[j] = acc_ref[j] * alpha + _dot(vta_ref[c], p.astype(bf16))
        m_ref[j] = m_new

    def fin(it):
        @pl.when(it % n_chunks == n_chunks - 1)
        def _():
            g = it // n_chunks
            for j in range(GH):
                r0 = pl.multiple_of((g * GH + j) * dh, dh)
                ota_ref[pl.ds(r0, dh), :] = (acc_ref[j] / l_ref[j]).astype(bf16)
            m_ref[...] = jnp.full(m_ref.shape, -jnp.inf, jnp.float32)
            l_ref[...] = jnp.zeros(l_ref.shape, jnp.float32)
            acc_ref[...] = jnp.zeros(acc_ref.shape, jnp.float32)

    def a_body(i2, z):
        it = 2 * i2
        for j in range(GH):
            qk(it + 1, 1, j)
            sm(it, 0, j)
        for j in range(GH):
            qk(jnp.minimum(it + 2, n_it - 1), 0, j)
            sm(it + 1, 1, j)
        fin(it + 1)
        return z

    def a_out_copy(t):
        return pltpu.make_async_copy(
            oa_ref.at[t],
            o_hbm.at[pl.ds(pl.multiple_of(t * TA, TA), TA), pl.ds(0, D)],
            out_sems.at[t])

    def a_tile(t, z):
        def a_proj(r, z2):
            r0 = pl.multiple_of(r * RP, RP)
            xa_t = xa_ref[pl.ds(pl.multiple_of(t * TA + r0, RP), RP), :]
            q = (_dot(xa_t, wq_ref[...]) * qscale).astype(bf16)
            for g in range(ng):
                qa_ref[g, pl.ds(r0, RP), :] = q[:, g * GH * dh:(g + 1) * GH * dh]
            return z2

        lax.fori_loop(0, TA // RP, a_proj, 0)
        for j in range(GH):
            qk(0, 0, j)
        lax.fori_loop(0, n_it // 2, a_body, 0)

        @pl.when(t == 0)
        def _():
            later[0].wait()

        oa_ref[t] = _dot_tn(ota_ref[...], woa_ref[...]).astype(bf16)
        a_out_copy(t).start()
        return z

    lax.fori_loop(0, S // TA, a_tile, 0)

    later[1].wait()
    later[2].wait()
    later[3].wait()
    nk = WIN + QB
    nb = TB // QB
    r_i = lax.broadcasted_iota(jnp.int32, (nk, GH * QB), 0)
    c_i = lax.broadcasted_iota(jnp.int32, (nk, GH * QB), 1) % QB
    band = (r_i > c_i) & (r_i <= c_i + WIN)
    bbufs = ((bsa_ref, bma_ref), (bsb_ref, bmb_ref))

    def b_qk(g, b, slot):
        s_r, m_r = bbufs[slot]
        k4 = kb_ref[g, b * QB:b * QB + nk, :]
        s = _dot_nt(k4, qm_ref[g, b])
        s = jnp.where(mask_ref[b] > 0.0, s, NEG)
        s_r[...] = s
        m_r[...] = jnp.max(s, axis=0, keepdims=True)

    def b_sm(g, b, slot):
        s_r, m_r = bbufs[slot]
        for j in range(GH):
            p = jnp.exp2(s_r[:, j * QB:(j + 1) * QB] - m_r[:, j * QB:(j + 1) * QB])
            l = jnp.sum(p, axis=0, keepdims=True)
            r0 = pl.multiple_of((g * GH + j) * dh, dh)
            vt = vtb_ref[pl.ds(r0, dh), b * QB:b * QB + nk]
            o = _dot(vt, p.astype(bf16)) / l
            otb_ref[pl.ds(r0, dh), b * QB:(b + 1) * QB] = o.astype(bf16)

    def b_body(g, z):
        for b in range(nb):
            if b + 1 < nb:
                b_qk(g, b + 1, (b + 1) % 2)
            else:
                b_qk(jnp.minimum(g + 1, ng - 1), 0, 0)
            b_sm(g, b, b % 2)
        return z

    def b_out_copy(i):
        return pltpu.make_async_copy(
            ob_ref.at[i],
            o_hbm.at[pl.ds(pl.multiple_of(i * TB, TB), TB), pl.ds(D, D)],
            out_sems.at[S // TA + i])

    def b_tile(i, z):
        xb_t = xb_ref[pl.ds(pl.multiple_of(i * TB, TB), TB), :]
        qkv = _dot(xb_t, wqkv_ref[...])
        qf = qkv[:, 0:D] * qscale
        kb = qkv[:, D:2 * D].astype(bf16)
        for g in range(ng):
            kb_ref[g, WIN:WIN + TB, :] = kb[:, g * GH * dh:(g + 1) * GH * dh]
            qg = qf[:, g * GH * dh:(g + 1) * GH * dh]
            for j in range(GH):
                piece = jnp.where((lane128 >= dh * j) & (lane128 < dh * (j + 1)),
                                  qg, 0.0).astype(bf16)
                for b in range(nb):
                    qm_ref[g, b, j * QB:(j + 1) * QB, :] = piece[b * QB:(b + 1) * QB]
        vtb_ref[:, WIN:WIN + TB] = qkv[:, 2 * D:3 * D].T.astype(bf16)

        for b in range(nb):
            valid = band & (r_i + (i * TB + b * QB) >= WIN)
            mask_ref[b] = jnp.where(valid, 1.0, 0.0)
        b_qk(0, 0, 0)
        lax.fori_loop(0, ng, b_body, 0)

        ob_ref[i] = _dot_tn(otb_ref[...], wob_ref[...]).astype(bf16)
        b_out_copy(i).start()
        kb_ref[:, 0:WIN, :] = kb_ref[:, TB:TB + WIN, :]
        vtb_ref[:, 0:WIN] = vtb_ref[:, TB:TB + WIN]
        return z

    lax.fori_loop(0, S // TB, b_tile, 0)

    for t in range(S // TA):
        a_out_copy(t).wait()
    for i in range(S // TB):
        b_out_copy(i).wait()


@jax.jit
def pallas_concat_heads__grouped_kv_mqa__sliding_block__prompt_kernel(
    A_x: jax.Array,
    A_wq: jax.Array,
    A_wk: jax.Array,
    A_wv: jax.Array,
    A_wo: jax.Array,
    B_x: jax.Array,
    B_wqkv: jax.Array,
    B_wo: jax.Array,
):
    B, S, D = A_x.shape
    dh = D // H
    ng = H // GH
    assert B == 1 and GH * dh == 128 and S % TA == 0 and S % TB == 0
    bf16 = jnp.bfloat16
    f32 = jnp.float32
    hbm = pl.BlockSpec(memory_space=pl.ANY)
    V = pltpu.VMEM
    out = pl.pallas_call(
        lambda *refs: _kernel(*refs, S=S, D=D),
        in_specs=[hbm] * 8,
        out_specs=hbm,
        out_shape=jax.ShapeDtypeStruct((S, 2 * D), A_x.dtype),
        scratch_shapes=[
            V((S, D), bf16), V((D, D), bf16), V((dh, D), bf16), V((dh, D), bf16),
            V((D, D), bf16), V((S, D), bf16), V((D, 3 * D), bf16), V((D, D), bf16),
            pltpu.SemaphoreType.DMA((2 + S // XC + 5,)),
            pltpu.SemaphoreType.DMA((S // TA + S // TB,)),
            V((GH, S, GH * dh), bf16),
            V((S // KC, dh, KC), bf16),
            V((ng, TA, GH * dh), bf16),
            V((D, TA), bf16),
            V((S // TA, TA, D), bf16),
            V((GH, KC, TA), f32), V((GH, 1, TA), f32),
            V((GH, KC, TA), f32), V((GH, 1, TA), f32),
            V((GH, 1, TA), f32), V((GH, 1, TA), f32), V((GH, dh, TA), f32),
            V((ng, TB // QB, GH * QB, GH * dh), bf16),
            V((ng, WIN + TB, GH * dh), bf16),
            V((D, WIN + TB), bf16),
            V((D, TB), bf16),
            V((S // TB, TB, D), bf16),
            V((TB // QB, WIN + QB, GH * QB), f32),
            V((WIN + QB, GH * QB), f32), V((1, GH * QB), f32),
            V((WIN + QB, GH * QB), f32), V((1, GH * QB), f32),
        ],
        compiler_params=pltpu.CompilerParams(vmem_limit_bytes=110 * 1024 * 1024),
    )(A_x.reshape(S, D), A_wq, A_wk.T, A_wv.T, A_wo,
      B_x.reshape(S, D), B_wqkv, B_wo)
    return out.reshape(B, S, 2 * D)
```

```python
import math

import jax
import jax.numpy as jnp
from jax import lax
import jax.experimental.pallas as pl
import jax.experimental.pallas.tpu as pltpu

H = 32
WIN = 256
NEG = -1e9
GH = 4
TA = 1024
KC = 128
RP = 256
XC = 512
TB = 512
QB = 128

_NT = (((1,), (1,)), ((), ()))
_TN = (((0,), (0,)), ((), ()))


def _dot(a, b):
    return jnp.dot(a, b, preferred_element_type=jnp.float32)


def _dot_nt(a, b):
    return lax.dot_general(a, b, _NT, preferred_element_type=jnp.float32)


def _dot_tn(a, b):
    return lax.dot_general(a, b, _TN, preferred_element_type=jnp.float32)


def _kernel(xa_hbm, wq_hbm, wkt_hbm, wvt_hbm, woa_hbm, xb_hbm, wqkv_hbm, wob_hbm,
            o_hbm,
            xa_ref, wq_ref, wkt_ref, wvt_ref, woa_ref, xb_ref, wqkv_ref, wob_ref,
            in_sems, out_sems,
            ks_ref, vta_ref, qa_ref, ota_ref, oa_ref,
            sa_ref, cma_ref, sb_ref, cmb_ref, m_ref, l_ref, acc_ref,
            qm_ref, kb_ref, vtb_ref, otb_ref, ob_ref, mask_ref,
            bsa_ref, bma_ref, bsb_ref, bmb_ref,
            *, S, D):
    dh = D // H
    ng = H // GH
    n_chunks = S // KC
    n_xc = S // XC
    qscale = (dh ** -0.5) * math.log2(math.e)
    bf16 = jnp.bfloat16
    lane128 = lax.broadcasted_iota(jnp.int32, (1, GH * dh), 1)

    first = [pltpu.make_async_copy(wkt_hbm, wkt_ref, in_sems.at[0]),
             pltpu.make_async_copy(wvt_hbm, wvt_ref, in_sems.at[1])]
    xcp = [pltpu.make_async_copy(xa_hbm.at[c * XC:(c + 1) * XC],
                                 xa_ref.at[c * XC:(c + 1) * XC],
                                 in_sems.at[2 + c]) for c in range(n_xc)]
    base = 2 + n_xc
    wq_cp = pltpu.make_async_copy(wq_hbm, wq_ref, in_sems.at[base])
    later = [pltpu.make_async_copy(h, v, in_sems.at[base + 1 + i])
             for i, (h, v) in enumerate(((woa_hbm, woa_ref), (xb_hbm, xb_ref),
                                         (wqkv_hbm, wqkv_ref), (wob_hbm, wob_ref)))]
    for cp in first + xcp + [wq_cp]:
        cp.start()

    row = lax.broadcasted_iota(jnp.int32, (dh, GH * dh), 0)
    col = lax.broadcasted_iota(jnp.int32, (dh, GH * dh), 1)
    for cp in first:
        cp.wait()
    for c in range(n_xc):
        xcp[c].wait()
        xc = xa_ref[c * XC:(c + 1) * XC, :]
        k = _dot_nt(xc, wkt_ref[...]).astype(bf16)
        vt = _dot_nt(wvt_ref[...], xc).astype(bf16)
        for j in range(GH):
            ej = jnp.where(col == row + dh * j, 1.0, 0.0).astype(bf16)
            ks_ref[j, c * XC:(c + 1) * XC, :] = _dot(k, ej).astype(bf16)
        for cc in range(XC // KC):
            vta_ref[c * (XC // KC) + cc] = vt[:, cc * KC:(cc + 1) * KC]
    for cp in later:
        cp.start()
    kb_ref[:, 0:WIN, :] = jnp.zeros((ng, WIN, GH * dh), bf16)
    vtb_ref[:, 0:WIN] = jnp.zeros((D, WIN), bf16)
    m_ref[...] = jnp.full(m_ref.shape, -jnp.inf, jnp.float32)
    l_ref[...] = jnp.zeros(l_ref.shape, jnp.float32)
    acc_ref[...] = jnp.zeros(acc_ref.shape, jnp.float32)
    wq_cp.wait()

    n_it = ng * n_chunks
    bufs = ((sa_ref, cma_ref), (sb_ref, cmb_ref))

    def qk(it, slot, j):
        s_r, cm_r = bufs[slot]
        g = it // n_chunks
        c = it % n_chunks
        kj = ks_ref[j, pl.ds(pl.multiple_of(c * KC, KC), KC), :]
        s = _dot_nt(kj, qa_ref[g])
        s_r[j] = s
        cm_r[j] = jnp.max(s, axis=0, keepdims=True)

    def sm(it, slot, j):
        s_r, cm_r = bufs[slot]
        c = it % n_chunks
        m = m_ref[j]
        m_new = jnp.maximum(m, cm_r[j])
        p = jnp.exp2(s_r[j] - m_new)
        alpha = jnp.exp2(m - m_new)
        l_ref[j] = l_ref[j] * alpha + jnp.sum(p, axis=0, keepdims=True)
        acc_ref[j] = acc_ref[j] * alpha + _dot(vta_ref[c], p.astype(bf16))
        m_ref[j] = m_new

    def fin(it):
        @pl.when(it % n_chunks == n_chunks - 1)
        def _():
            g = it // n_chunks
            for j in range(GH):
                r0 = pl.multiple_of((g * GH + j) * dh, dh)
                ota_ref[pl.ds(r0, dh), :] = (acc_ref[j] / l_ref[j]).astype(bf16)
            m_ref[...] = jnp.full(m_ref.shape, -jnp.inf, jnp.float32)
            l_ref[...] = jnp.zeros(l_ref.shape, jnp.float32)
            acc_ref[...] = jnp.zeros(acc_ref.shape, jnp.float32)

    def a_body(i2, z):
        it = 2 * i2
        for j in range(GH):
            qk(it + 1, 1, j)
            sm(it, 0, j)
        for j in range(GH):
            qk(jnp.minimum(it + 2, n_it - 1), 0, j)
            sm(it + 1, 1, j)
        fin(it + 1)
        return z

    def a_out_copy(t):
        return pltpu.make_async_copy(
            oa_ref.at[t],
            o_hbm.at[pl.ds(pl.multiple_of(t * TA, TA), TA), pl.ds(0, D)],
            out_sems.at[t])

    def a_tile(t, z):
        def a_proj(r, z2):
            r0 = pl.multiple_of(r * RP, RP)
            xa_t = xa_ref[pl.ds(pl.multiple_of(t * TA + r0, RP), RP), :]
            q = (_dot(xa_t, wq_ref[...]) * qscale).astype(bf16)
            for g in range(ng):
                qa_ref[g, pl.ds(r0, RP), :] = q[:, g * GH * dh:(g + 1) * GH * dh]
            return z2

        lax.fori_loop(0, TA // RP, a_proj, 0)
        for j in range(GH):
            qk(0, 0, j)
        lax.fori_loop(0, n_it // 2, a_body, 0)

        @pl.when(t == 0)
        def _():
            later[0].wait()

        oa_ref[t] = _dot_tn(ota_ref[...], woa_ref[...]).astype(bf16)
        a_out_copy(t).start()
        return z

    lax.fori_loop(0, S // TA, a_tile, 0)

    later[1].wait()
    later[2].wait()
    later[3].wait()
    nk = WIN + QB
    nb = TB // QB
    r_i = lax.broadcasted_iota(jnp.int32, (nk, GH * QB), 0)
    c_i = lax.broadcasted_iota(jnp.int32, (nk, GH * QB), 1) % QB
    band = (r_i > c_i) & (r_i <= c_i + WIN)
    bbufs = ((bsa_ref, bma_ref), (bsb_ref, bmb_ref))

    def b_qk(g, b, slot):
        s_r, m_r = bbufs[slot]
        k4 = kb_ref[g, b * QB:b * QB + nk, :]
        s = _dot_nt(k4, qm_ref[g, b])
        if b == 0:
            s = jnp.where(mask_ref[b] > 0.0, s, NEG)
        else:
            s = jnp.concatenate([
                jnp.where(mask_ref[b, 0:QB] > 0.0, s[0:QB], NEG),
                s[QB:WIN],
                jnp.where(mask_ref[b, WIN:nk] > 0.0, s[WIN:nk], NEG)], axis=0)
        s_r[...] = s
        m_r[...] = jnp.max(s, axis=0, keepdims=True)

    def b_sm(g, b, slot):
        s_r, m_r = bbufs[slot]
        for j in range(GH):
            p = jnp.exp2(s_r[:, j * QB:(j + 1) * QB] - m_r[:, j * QB:(j + 1) * QB])
            l = jnp.sum(p, axis=0, keepdims=True)
            r0 = pl.multiple_of((g * GH + j) * dh, dh)
            vt = vtb_ref[pl.ds(r0, dh), b * QB:b * QB + nk]
            o = _dot(vt, p.astype(bf16)) / l
            otb_ref[pl.ds(r0, dh), b * QB:(b + 1) * QB] = o.astype(bf16)

    def b_body(g, z):
        for b in range(nb):
            if b + 1 < nb:
                b_qk(g, b + 1, (b + 1) % 2)
            else:
                b_qk(jnp.minimum(g + 1, ng - 1), 0, 0)
            b_sm(g, b, b % 2)
        return z

    def b_out_copy(i):
        return pltpu.make_async_copy(
            ob_ref.at[i],
            o_hbm.at[pl.ds(pl.multiple_of(i * TB, TB), TB), pl.ds(D, D)],
            out_sems.at[S // TA + i])

    def b_tile(i, z):
        xb_t = xb_ref[pl.ds(pl.multiple_of(i * TB, TB), TB), :]
        qkv = _dot(xb_t, wqkv_ref[...])
        qf = qkv[:, 0:D] * qscale
        kb = qkv[:, D:2 * D].astype(bf16)
        for g in range(ng):
            kb_ref[g, WIN:WIN + TB, :] = kb[:, g * GH * dh:(g + 1) * GH * dh]
            qg = qf[:, g * GH * dh:(g + 1) * GH * dh]
            for j in range(GH):
                piece = jnp.where((lane128 >= dh * j) & (lane128 < dh * (j + 1)),
                                  qg, 0.0).astype(bf16)
                for b in range(nb):
                    qm_ref[g, b, j * QB:(j + 1) * QB, :] = piece[b * QB:(b + 1) * QB]
        vtb_ref[:, WIN:WIN + TB] = qkv[:, 2 * D:3 * D].T.astype(bf16)

        for b in range(nb):
            valid = band & (r_i + (i * TB + b * QB) >= WIN)
            mask_ref[b] = jnp.where(valid, 1.0, 0.0)
        b_qk(0, 0, 0)
        lax.fori_loop(0, ng, b_body, 0)

        ob_ref[i] = _dot_tn(otb_ref[...], wob_ref[...]).astype(bf16)
        b_out_copy(i).start()
        kb_ref[:, 0:WIN, :] = kb_ref[:, TB:TB + WIN, :]
        vtb_ref[:, 0:WIN] = vtb_ref[:, TB:TB + WIN]
        return z

    lax.fori_loop(0, S // TB, b_tile, 0)

    for t in range(S // TA):
        a_out_copy(t).wait()
    for i in range(S // TB):
        b_out_copy(i).wait()


@jax.jit
def pallas_concat_heads__grouped_kv_mqa__sliding_block__prompt_kernel(
    A_x: jax.Array,
    A_wq: jax.Array,
    A_wk: jax.Array,
    A_wv: jax.Array,
    A_wo: jax.Array,
    B_x: jax.Array,
    B_wqkv: jax.Array,
    B_wo: jax.Array,
):
    B, S, D = A_x.shape
    dh = D // H
    ng = H // GH
    assert B == 1 and GH * dh == 128 and S % TA == 0 and S % TB == 0
    bf16 = jnp.bfloat16
    f32 = jnp.float32
    hbm = pl.BlockSpec(memory_space=pl.ANY)
    V = pltpu.VMEM
    out = pl.pallas_call(
        lambda *refs: _kernel(*refs, S=S, D=D),
        in_specs=[hbm] * 8,
        out_specs=hbm,
        out_shape=jax.ShapeDtypeStruct((S, 2 * D), A_x.dtype),
        scratch_shapes=[
            V((S, D), bf16), V((D, D), bf16), V((dh, D), bf16), V((dh, D), bf16),
            V((D, D), bf16), V((S, D), bf16), V((D, 3 * D), bf16), V((D, D), bf16),
            pltpu.SemaphoreType.DMA((2 + S // XC + 5,)),
            pltpu.SemaphoreType.DMA((S // TA + S // TB,)),
            V((GH, S, GH * dh), bf16),
            V((S // KC, dh, KC), bf16),
            V((ng, TA, GH * dh), bf16),
            V((D, TA), bf16),
            V((S // TA, TA, D), bf16),
            V((GH, KC, TA), f32), V((GH, 1, TA), f32),
            V((GH, KC, TA), f32), V((GH, 1, TA), f32),
            V((GH, 1, TA), f32), V((GH, 1, TA), f32), V((GH, dh, TA), f32),
            V((ng, TB // QB, GH * QB, GH * dh), bf16),
            V((ng, WIN + TB, GH * dh), bf16),
            V((D, WIN + TB), bf16),
            V((D, TB), bf16),
            V((S // TB, TB, D), bf16),
            V((TB // QB, WIN + QB, GH * QB), f32),
            V((WIN + QB, GH * QB), f32), V((1, GH * QB), f32),
            V((WIN + QB, GH * QB), f32), V((1, GH * QB), f32),
        ],
        compiler_params=pltpu.CompilerParams(vmem_limit_bytes=110 * 1024 * 1024),
    )(A_x.reshape(S, D), A_wq, A_wk.T, A_wv.T, A_wo,
      B_x.reshape(S, D), B_wqkv, B_wo)
    return out.reshape(B, S, 2 * D)
```
